```python
import os as _os
_os.environ.setdefault("JAX_PLATFORMS", "cpu")
import jax
import jax.numpy as jnp

def _softmax(x, axis=-1):
    return jax.nn.softmax(x, axis=axis)
def _gelu(x):
    return jax.nn.gelu(x, approximate=True)
def _silu(x):
    return jax.nn.silu(x)
def _sigmoid(x):
    return jax.nn.sigmoid(x)
def _layernorm(x, axis=-1, eps=1e-5):
    m = jnp.mean(x, axis=axis, keepdims=True)
    v = jnp.var(x, axis=axis, keepdims=True)
    return (x - m) / jnp.sqrt(v + eps)
def _scatter_add(tgt, idx, src, axis=0):
    return tgt.at[idx].add(src)
def _segment_sum(src, seg, n):
    return jax.ops.segment_sum(src, seg, n)
class _Rng:
    def __init__(self, key):
        self._k = key
    def _next(self):
        self._k, sub = jax.random.split(self._k)
        return sub
    def normal(self, shape):
        return jax.random.normal(self._next(), shape, dtype=jnp.bfloat16)
    def randint(self, lo, hi, shape):
        return jax.random.randint(self._next(), shape, lo, hi, dtype=jnp.int32)
    def uniform(self, shape, lo=0.0, hi=1.0):
        return jax.random.uniform(self._next(), shape, jnp.bfloat16, lo, hi)
    def permutation(self, n):
        return jax.random.permutation(self._next(), n)


kernel_name = 'interleave_layers__ssm_conv_h3__geglu_ffn__prompt'

def setup_inputs():
    _rng = _Rng(jax.random.key(int.from_bytes(__import__("os").urandom(4), "little")))
    _w = (lambda a: (lambda t: t.astype(jnp.bfloat16) if jnp.issubdtype(t.dtype, jnp.floating) else t)(jnp.asarray(a)))
    def _A_setup():
        B, S, D = 1, 2048, 448
        ks = 4
        return {
            "q": _w((lambda *s: _rng.normal(s) * 0.05)(B, S, D)),
            "k": _w((lambda *s: _rng.normal(s) * 0.8)(B, S, D)),
            "v": _w((lambda *s: _rng.normal(s) * 0.8)(B, S, D)),
            "shift_k": _w((lambda *s: _rng.normal(s) * 0.8)(D, ks) * 0.5),
            "ssm_k": _w((lambda *s: _rng.normal(s) * 0.8)(D, S) * (1.0 / S ** 0.5)),
            "ssm_D": _w((lambda *s: _rng.normal(s) * 0.8)(D)),
        }
    _A_in = _A_setup()

    def _B_setup():
        B, S, D, F = 1, 2048, 448, 1792
        return {
            "x": _w((lambda *s: _rng.normal(s) * 0.05)(B, S, D)),
            "w_gate": _w((lambda *s: _rng.normal(s) * 0.1)(D, F)),
            "w_up": _w((lambda *s: _rng.normal(s) * 0.1)(D, F)),
            "w_down": _w((lambda *s: _rng.normal(s) * 0.1)(F, D)),
        }
    _B_in = _B_setup()

    return {
        "A_q": _A_in["q"],
        "A_k": _A_in["k"],
        "A_v": _A_in["v"],
        "A_shift_k": _A_in["shift_k"],
        "A_ssm_k": _A_in["ssm_k"],
        "A_ssm_D": _A_in["ssm_D"],
        "B_x": _B_in["x"],
        "B_w_gate": _B_in["w_gate"],
        "B_w_up": _B_in["w_up"],
        "B_w_down": _B_in["w_down"],
    }

def reference(A_q, A_k, A_v, A_shift_k, A_ssm_k, A_ssm_D, B_x, B_w_gate, B_w_up, B_w_down):
    def _A_ref(q, k, v, shift_k, ssm_k, ssm_D):
        B, S, D = q.shape
        ks = shift_k.shape[-1]
        k_pad = jnp.pad(k, ((0, 0), (ks - 1, 0), (0, 0)))
        k_shift = jnp.zeros_like(k)
        for t in range(ks):
            k_shift = k_shift + k_pad[:, t:t + S, :] * shift_k[:, ks - 1 - t][None, None, :]
        kv = k_shift * v
        L = 2 * S
        kv_pad = jnp.pad(kv, ((0, 0), (0, S), (0, 0)))
        kf_pad = jnp.pad(ssm_k, ((0, 0), (0, S)))
        kv_f = (lambda x, axes=(-2,-1): jnp.fft.rfft2(x.astype(jnp.float32), axes=axes))(kv_pad[:, None, :, :], axes=(1, 2))
        kf_f = (lambda x, axes=(-2,-1): jnp.fft.rfft2(x.astype(jnp.float32), axes=axes))(kf_pad[:, None, :], axes=(1, 2))
        kf_f = (lambda x, *d: x.transpose(*d))(kf_f, 1, 2, 0)
        y_f = kv_f * kf_f[None, :, :, :]
        y = (lambda x, s, axes=(-2,-1): jnp.fft.irfft2(x, s=s, axes=axes).astype(jnp.bfloat16))(y_f, (1, L), axes=(1, 2))[:, 0, :S, :]
        y = y + kv * ssm_D[None, None, :]
        return q * y

    def _B_ref(x, w_gate, w_up, w_down):
        return (_gelu(x @ w_gate) * (x @ w_up)) @ w_down

    x = A_q
    x = x + _A_ref(_layernorm(x, axis=-1), A_k, A_v, A_shift_k, A_ssm_k, A_ssm_D)
    x = x + _B_ref(_layernorm(x, axis=-1), B_w_gate, B_w_up, B_w_down)
    x = x + _A_ref(_layernorm(x, axis=-1), A_k, A_v, A_shift_k, A_ssm_k, A_ssm_D)
    x = x + _B_ref(_layernorm(x, axis=-1), B_w_gate, B_w_up, B_w_down)
    return x
```

```python
import contextlib
import functools
import itertools

import numpy as np
import jax
import jax.numpy as jnp
import jax.experimental.pallas as pl
import jax.experimental.pallas.tpu as pltpu

BF16, F32, U32 = jnp.bfloat16, jnp.float32, jnp.uint32
S, D, F = 2048, 448, 1792
L = 128
NB = S // L
G = 4 * L
NG = S // G
KQ = D // 4
FH = F // 2
H = D // 2
EPS = 1e-5
GELU_C0 = float(np.sqrt(2.0 / np.pi))
GELU_C1 = GELU_C0 * 0.044715


def _dft_tables():
    j = np.arange(L)[:, None]
    m = np.arange(L)[None, :]
    th = 2.0 * np.pi * j * (m + 1.0 / 3.0) / L
    fwd = np.concatenate([np.cos(th - np.pi / 6), np.sin(th)], axis=1)
    scale = (2.0 / np.sqrt(3.0)) ** 3 / L
    inv = np.concatenate([np.cos(th + np.pi / 6).T, np.sin(th).T], axis=1) * scale
    return np.concatenate([fwd, inv], axis=0).astype(BF16)


def _dot(a, b):
    return jnp.dot(a, b, preferred_element_type=F32)


_PRE_A = (lambda a, b, c, d: a + d, lambda a, b, c, d: c + d, lambda a, b, c, d: a, lambda a, b, c, d: d,
          lambda a, b, c, d: a + b, lambda a, b, c, d: c - a, lambda a, b, c, d: b - d)
_PRE_B = (lambda a, b, c, d: a + d, lambda a, b, c, d: a, lambda a, b, c, d: b - d, lambda a, b, c, d: c - a,
          lambda a, b, c, d: d, lambda a, b, c, d: a + b, lambda a, b, c, d: c + d)


def _post(m1, m2, m3, m4, m5, m6, m7):
    return (m1 + m4 - m5 + m7, m3 + m5, m2 + m4, m1 - m2 + m3 + m6)


def _pre2(pre, blk):
    for f in pre:
        outer = [f(blk[a][b], blk[a][2 + b], blk[2 + a][b], blk[2 + a][2 + b]) for a in range(2) for b in range(2)]
        for g in pre:
            yield g(*outer)


def _pack_rows(even, odd):
    n, w = even.shape
    return pltpu.bitcast(jnp.concatenate([even, odd], axis=1).astype(BF16).reshape(2 * n, w), U32)


def _unpack_rows(x):
    u = pltpu.bitcast(x, U32)
    return pltpu.bitcast(u << 16, F32), pltpu.bitcast(u & np.uint32(0xFFFF0000), F32)


def _geglu(g, u):
    t = jnp.tanh(g * (GELU_C0 + GELU_C1 * (g * g)))
    return (g * u) * (0.5 + 0.5 * t)


def _causal(k, u, init=None):
    acc = [kk * u[0] for kk in k]
    if init is not None:
        acc = [i + t for i, t in zip(init, acc)]
    for b in range(1, len(k)):
        for a in range(b, len(k)):
            acc[a] = acc[a] + k[a - b] * u[b]
    return acc


def _causal_split(k, u):
    ke, ko, ue, uo = k[0::2], k[1::2], u[0::2], u[1::2]
    n = len(ke)
    p1 = _causal(ke, [a + b for a, b in zip(ue, uo)])
    even = _causal([-ke[0]] + [ko[i - 1] - ke[i] for i in range(1, n)], uo, p1)
    odd = _causal([b - a for a, b in zip(ke, ko)], ue, p1)
    return [v for pair in zip(even, odd) for v in pair]


def _spectral(w1, w2, u1, u2):
    t1 = _causal_split([w1[0]] + [w1[b] + w2[b - 1] for b in range(1, NB)], u1)
    w3 = [a - b for a, b in zip(w1, w2)]
    t2 = _causal_split([w2[0]] + [w2[b] - w3[b - 1] for b in range(1, NB)], u2)
    y1 = [a - b for a, b in zip(t1, t2)]
    t3 = _causal_split([w3[0]] + [w3[b] + w1[b - 1] for b in range(1, NB)], [a - b for a, b in zip(u1, u2)])
    return y1, [a - b for a, b in zip(t1, t3)]


def _interleave(*streams):
    done = [0] * len(streams)
    live = list(range(len(streams)))
    while live:
        i = min(live, key=lambda j: (done[j] + 0.5) / streams[j][1])
        try:
            next(streams[i][0])
            done[i] += 1
        except StopIteration:
            live.remove(i)


def make(RC=32, checks=False, CG=64, LAG=1, scopes=False, MIXW=1.3, flags=None, RPOS=20, PLAG=2, GW=1.1,
         ORD=(3, 1, 2, 4, 0, 6, 5), OPN=24, NGU=1, DP=(0, 4), short2=False, cstage=True, wt=0, dstage=True, WU=1):
    scope = jax.named_scope if scopes else (lambda n: contextlib.nullcontext())
    SUB = 16
    RB = 32
    NC = D // CG
    SEM_C, SEM_Q, SEM_O = 3, 3 + NC, 3 + NC + NG

    def kernel(q_h, k_h, v_h, sk_h, sm_h, sd_h, wg_h, wu_h, wd_h, dft_h, o_h,
               xs, kb, vb, smb, skb, sdb, wgb, wub, wdb, dft, par, f0, f1, f2, ys, xm, wa, xb, hb, wdc, dm, sem):
        def aligned(start, size):
            return pl.ds(start if isinstance(start, int) else pl.multiple_of(start, size), size)

        def conv_copies(c):
            rows = aligned(c * CG, CG)
            return [pltpu.make_async_copy(src.at[rows], dst.at[rows], sem.at[SEM_C + c])
                    for src, dst in ((sm_h, smb), (k_h, kb), (v_h, vb))]

        def q_copy(g):
            return pltpu.make_async_copy(q_h.at[:, pl.ds(g * G, G)], xs.at[g], sem.at[SEM_Q + g])

        def out_copy(g):
            return pltpu.make_async_copy(xs.at[g], o_h.at[:, aligned(g * G, G)], sem.at[SEM_O + g])

        small = [pltpu.make_async_copy(s, d, sem.at[0]) for s, d in ((sk_h, skb), (sd_h, sdb), (dft_h, dft))]
        w_copies = [pltpu.make_async_copy(s, d, sem.at[1]) for s, d in ((wg_h, wgb), (wu_h, wub))]
        wd_copy = pltpu.make_async_copy(wd_h, wdb, sem.at[2])
        for cp in (small + [cp for c in range(NC) for cp in conv_copies(c)] + w_copies + [wd_copy]
                   + [q_copy(g) for g in range(NG)]):
            cp.start()

        for i in range(49):
            xb[i, KQ // 2:, :] = jnp.zeros((L // 2 - KQ // 2, L), U32)

        with scope("small"):
            for cp in small:
                cp.wait()
            par[...] = jnp.concatenate([skb[...].astype(F32), sdb[...].astype(F32).reshape(1, D),
                                        jnp.zeros((3, D), F32)], axis=0).T

        def gated_input(rows):
            lane = jax.lax.broadcasted_iota(jnp.int32, (SUB // 2, L), 1)
            lane2 = jax.lax.broadcasted_iota(jnp.int32, (SUB, L), 1)
            pr = par[rows, :]
            sc = [jnp.broadcast_to(pr[:, j:j + 1], (SUB, L)) for j in range(4)]
            prev = [jnp.zeros((SUB // 2, L), U32)] * 3
            far = jnp.zeros((SUB, L), F32)
            kv = []
            for b in range(NB):
                if b % 2 == 0:
                    vt = vb[rows, b * L:(b + 2) * L].astype(F32)
                words = pltpu.bitcast(kb[rows, b * L:(b + 1) * L], U32)
                taps = [words]
                for j in range(1, 2 if short2 else 4):
                    r = pltpu.roll(words, j, 1)
                    taps.append(jnp.where(lane < j, prev[j - 1], r))
                    prev[j - 1] = r
                taps = [pltpu.bitcast(t, BF16).astype(F32) for t in taps]
                acc = sc[0] * taps[0] + sc[1] * taps[1]
                if short2:
                    r = pltpu.roll(sc[2] * taps[0] + sc[3] * taps[1], 2, 1)
                    acc, far = acc + jnp.where(lane2 < 2, far, r), r
                else:
                    acc = acc + sc[2] * taps[2] + sc[3] * taps[3]
                kv.append(acc * vt[:, (b % 2) * L:(b % 2 + 1) * L])
            return kv

        def conv_step(c, carry):
            for cp in conv_copies(c):
                cp.wait()
            with scope("conv"):
                pending = []
                for s in range(CG // SUB + LAG):
                    if s < CG // SUB:
                        r0 = c * CG + s * SUB
                        slabs = [aligned(r0 + 8 * e, 8) for e in range(SUB // 8)]
                        kf = _dot(jnp.concatenate([smb[sl, b * L:(b + 1) * L] for sl in slabs for b in range(NB)],
                                                  axis=0), dft[:L, :])
                        kv = gated_input(aligned(r0, SUB))
                        uf = _dot(jnp.concatenate([t[8 * e:8 * e + 8] for e in range(SUB // 8) for t in kv],
                                                  axis=0).astype(BF16), dft[:L, :])
                        if cstage:
                            st = (f0, f1, f2)[s % 3]
                            st[0], st[1] = kf, uf
                            kf, uf = st[c >> 10], st[(c >> 10) + 1]
                        y1, y2 = [], []
                        for e, sl in enumerate(slabs):
                            co = [[m[(e * NB + b) * 8:(e * NB + b + 1) * 8, h * L:(h + 1) * L] for b in range(NB)]
                                  for m in (kf, uf) for h in range(2)]
                            co[0][0] = co[0][0] + jnp.broadcast_to(par[sl, 4:5], (8, L)) * float(np.sqrt(0.75))
                            a, b = _spectral(*co)
                            y1 += a
                            y2 += b
                        pending.append((slabs, jnp.concatenate(
                            [jnp.concatenate(y1, axis=0), jnp.concatenate(y2, axis=0)], axis=1).astype(BF16)))
                    if s >= LAG:
                        slabs, spec = pending.pop(0)
                        y = _dot(spec, jnp.concatenate([dft[L:, :L], dft[L:, L:]], axis=0))
                        for e, sl in enumerate(slabs):
                            for b in range(NB):
                                ys[b // 4, sl, (b % 4) * L:(b % 4 + 1) * L] = y[(e * NB + b) * 8:(e * NB + b + 1) * 8]
            return carry

        with scope("conv_all"):
            jax.lax.fori_loop(0, NC, conv_step, 0)

        def weight_step(c, carry):
            def block(ref, fh, kq):
                w = ref[kq * KQ:(kq + 1) * KQ, aligned(fh * FH + c * L, L)]
                return jnp.concatenate([w, jnp.zeros((L - KQ, L), BF16)], axis=0).T
            blk = [[block(ref, fh, kq) for kq in range(4)] for ref in (wgb, wub) for fh in range(2)]
            quad = [wdb[i * H:(i + 1) * H, aligned(j * FH + c * L, L)] for i in range(2) for j in range(2)]
            for r in range(0, H, 16):
                rows = [jnp.concatenate(_unpack_rows(t[r:r + 16]), axis=0) for t in quad]
                for i, f in enumerate(_PRE_A):
                    v = f(*rows)
                    wdc[i, r // 2:r // 2 + 8, aligned(c * L, L)] = (
                        pltpu.bitcast(quad[3 * (i - 2)][r:r + 16], U32) if i in (2, 3) else _pack_rows(v[:8], v[8:]))
            for r in range(0, L, 16):
                rows = [[jnp.concatenate(_unpack_rows(t[r:r + 16]), axis=0) for t in row] for row in blk]
                for i, v in enumerate(_pre2(_PRE_A, rows)):
                    wa[i, aligned(c * (L // 2) + r // 2, 8), :] = _pack_rows(v[:8], v[8:])
            return carry

        with scope("wprep"):
            for cp in w_copies + [wd_copy]:
                cp.wait()
            jax.lax.fori_loop(0, FH // L, weight_step, 0, unroll=WU)

        def moments(tot, sq):
            mean = jnp.sum(tot, axis=0, keepdims=True) * (1.0 / D)
            var = jnp.maximum(jnp.sum(sq, axis=0, keepdims=True) * (1.0 / D) - mean * mean, 0.0)
            return mean, jax.lax.rsqrt(var + EPS)

        def input_stats(g, zero, st):
            tot = sq = None
            for r in range(0, D, RB):
                for e in range(r, r + RB, 8):
                    x = xs[g, e:e + 8, :].astype(F32)
                    tot, sq = (x, x * x) if tot is None else (tot + x, sq + x * x)
                yield
            st.extend(moments(tot, sq))

        def mix(g, zero, st):
            tot = sq = None
            for r in range(0, D, RB):
                for e in range(r, r + RB, 8):
                    x = xs[g + zero[0], e:e + 8, :].astype(F32)
                    x = x + ((x - st[0]) * st[1]) * ys[g, e:e + 8, :]
                    for j in range(4):
                        xm[g, j, e:e + 8, :] = x[:, j * L:(j + 1) * L]
                    tot, sq = (x, x * x) if tot is None else (tot + x, sq + x * x)
                yield
            st.extend(moments(tot, sq))

        def operands(g, zero, st, pin):
            for r in range(0, KQ, 16):
                z = [[jnp.concatenate([(xm[g + zero[1], j, pl.ds(kq * KQ + r + e, 8, stride=2), :]
                                        - st[2][:, j * L:(j + 1) * L]) * st[3][:, j * L:(j + 1) * L]
                                       for e in range(2)], axis=0) for j in range(4)] for kq in range(4)]
                for i, v in enumerate(_pre2(_PRE_B, z)):
                    xb[i, r // 2:r // 2 + 8, :] = _pack_rows(v[:8], v[8:])
                    if i % OPN == OPN - 1:
                        if pin:
                            pin(xb[i + zero[0], r // 2:r // 2 + 8, :])
                        yield

        def gate_up(release):
            for r in range(0, FH, RC):
                m = []
                for i in range(49):
                    m.append(_dot(pltpu.bitcast(wa[i, r // 2:(r + RC) // 2, :], BF16), pltpu.bitcast(xb[i], BF16)))
                    if i == RPOS:
                        release(m[-1])
                        yield
                inner = [_post(*m[7 * p:7 * p + 7]) for p in range(7)]
                for r1 in range(0, RC, 16):
                    h = {}
                    for e in range(4):
                        c = _post(*[inner[p][e][r1:r1 + 16] for p in range(7)])
                        h[e // 2, e % 2], h[e // 2, 2 + e % 2] = _geglu(c[0], c[2]), _geglu(c[1], c[3])
                    half = [jnp.concatenate([h[a, 2 * j], h[a, 2 * j + 1]], axis=1)
                            for a in range(2) for j in range(2)]
                    for i, f in enumerate(_PRE_B):
                        hb[i, r + r1:r + r1 + 16, :] = f(*half).astype(BF16)

        def down(g, zero, release):
            for n in range(2):
                cols = slice(n * L, (n + 1) * L)

                def emit(i, j, val):
                    rows = slice(i * H, (i + 1) * H)
                    xs[g, rows, (2 * j + n) * L:(2 * j + n + 1) * L] = (xm[g, 2 * j + n, rows, :] + val).astype(BF16)

                m = {}

                def old(i):
                    return dm[i + zero[0], :, cols] if dstage else m[i]
                for i in ORD:
                    m[i] = _dot(pltpu.bitcast(wdc[i], BF16), hb[i, :, cols])
                    release(m[i])
                    if dstage and i < 5:
                        dm[i, :, cols] = m[i]
                    if i == (1 if n else 0):
                        emit(1, 0, (m[1] if n else old(1)) + old(3))
                    if i == (4 if n else 0):
                        emit(0, 1, old(2) + (m[4] if n else old(4)))
                    if i == 6:
                        emit(0, 0, (old(3) - old(4)) + old(0) + m[6])
                    if i == 5:
                        emit(1, 1, (old(2) - old(1)) + old(0) + m[5])
                    yield

        with scope("prep0"):
            q_copy(0).wait()
            first = jnp.minimum(pl.program_id(0), 0)
            zero, st = (first >> 10, first >> 11), []
            for _ in itertools.chain(input_stats(first, zero, st), mix(first, zero, st),
                                     operands(first, zero, st, None)):
                pass
            for g in range(1, NG):
                q_copy(g).wait()

        def ffn_step(i, carry):
            g, nxt = i & (NG - 1), (i + 1) & (NG - 1)
            zero = (i >> 10, i >> 11)
            clock, queue, st = [0], [], []

            def release_xs(v):
                xs[zero[0] + NG, :8, :L] = v[:8, :L].astype(BF16)

            def release_xm(v):
                xm[zero[0] + NG, 0, :8, :] = v[:8, :L]

            active = [release_xs]

            def after_product(v):
                active[0](v)
                clock[0] += 1
                while queue and queue[0][0] <= clock[0]:
                    hb[zero[0] + 7, :8, :L] = pltpu.bitcast(queue.pop(0)[1], F32).astype(BF16)

            with scope("ffn"):
                stages = [input_stats(nxt, zero, st), mix(nxt, zero, st)]
                _interleave((gate_up(release_xs), FH // RC),
                            (itertools.chain(*stages[:NGU]), max(NGU, 1) * (D // RB) * GW))
                dn, left = down(g, zero, after_product), 14
                for j in range(NGU, 2):
                    _interleave((itertools.islice(dn, DP[j]), DP[j]), (stages[j], D // RB))
                    left -= DP[j]
                active[0] = release_xm
                _interleave((dn, left), (operands(nxt, zero, st, lambda v: queue.append((clock[0] + PLAG, v))),
                                         (49 // OPN) * (KQ // 16) * MIXW))

            @pl.when(i >= NG)
            def _():
                out_copy(g).start()
            return carry

        jax.lax.fori_loop(0, 2 * NG, ffn_step, 0)
        with scope("tail"):
            for g in range(NG):
                out_copy(g).wait()

    def fn(A_q, A_k, A_v, A_shift_k, A_ssm_k, A_ssm_D, B_x, B_w_gate, B_w_up, B_w_down):
        hbm = pl.BlockSpec(memory_space=pltpu.MemorySpace.HBM)
        out = pl.pallas_call(
            kernel,
            out_shape=jax.ShapeDtypeStruct((D, S), BF16),
            grid=(1,),
            in_specs=[hbm] * 10,
            out_specs=hbm,
            scratch_shapes=[
                pltpu.VMEM((NG + 1, D, G), BF16),
                pltpu.VMEM((D, S), BF16), pltpu.VMEM((D, S), BF16), pltpu.VMEM((D, S), BF16),
                pltpu.VMEM((4, D), BF16), pltpu.VMEM((D,), BF16),
                pltpu.VMEM((D, F), BF16), pltpu.VMEM((D, F), BF16), pltpu.VMEM((D, F), BF16),
                pltpu.VMEM((2 * L, 2 * L), BF16),
                pltpu.VMEM((D, 8), F32),
                *[pltpu.VMEM((2, NB * SUB, 2 * L), F32)] * 3,
                pltpu.VMEM((NG, D, G), F32), pltpu.VMEM((NG + 1, 4, D, L), F32),
                pltpu.VMEM((49, FH // 2, L), U32), pltpu.VMEM((49, L // 2, L), U32),
                pltpu.VMEM((8, FH, 2 * L), BF16), pltpu.VMEM((7, H // 2, FH), U32),
                pltpu.VMEM((5, H, 2 * L), F32),
                pltpu.SemaphoreType.DMA((SEM_O + NG,)),
            ],
            compiler_params=pltpu.CompilerParams(vmem_limit_bytes=100 * 2**20, disable_bounds_checks=not checks,
                                                 disable_semaphore_checks=not checks, flags=flags),
        )(A_q[0].T, A_k[0].T, A_v[0].T, A_shift_k.T, A_ssm_k, A_ssm_D, B_w_gate, B_w_up, B_w_down.T, _dft_tables())
        return out.T[None]

    return fn


@jax.jit
def pallas_interleave_layers__ssm_conv_h3__geglu_ffn__prompt_kernel(
        A_q, A_k, A_v, A_shift_k, A_ssm_k, A_ssm_D, B_x, B_w_gate, B_w_up, B_w_down):
    return make(**dict())(A_q, A_k, A_v, A_shift_k, A_ssm_k, A_ssm_D, B_x, B_w_gate, B_w_up, B_w_down)
```

```python
import functools
import itertools

import numpy as np
import jax
import jax.numpy as jnp
import jax.experimental.pallas as pl
import jax.experimental.pallas.tpu as pltpu

BF16, F32, U32 = jnp.bfloat16, jnp.float32, jnp.uint32
S, D, F = 2048, 448, 1792
L = 128
NB = S // L
G = 4 * L
NG = S // G
KQ = D // 4
H, FH = D // 2, F // 2
SUB = 16
RC = 64
RB = 32
CONV_CHUNKS = (0, 16, 48, 112, 224, 448)
EPS = 1e-5

GELU_IN = float((np.sqrt(2.0 / np.pi) * 0.044715) ** (1.0 / 3.0))
GELU_LIN = float(np.sqrt(2.0 / np.pi) / GELU_IN)
GELU_OUT = 0.5 / GELU_IN ** 2

_LEFT = (lambda x: x(0) + x(3), lambda x: x(2) + x(3), lambda x: x(0), lambda x: x(3),
         lambda x: x(0) + x(1), lambda x: x(2) - x(0), lambda x: x(1) - x(3))
_RIGHT = (lambda x: x(0) + x(3), lambda x: x(0), lambda x: x(1) - x(3), lambda x: x(2) - x(0),
          lambda x: x(3), lambda x: x(0) + x(1), lambda x: x(2) + x(3))
_ORDER = (3, 1, 2, 4, 0, 6, 5)


def _result_blocks(m):
    return (m[3] - m[4] + m[0] + m[6], m[2] + m[4], m[3] + m[1], m[2] - m[1] + m[0] + m[5])


def _two_level(operand, block, outer_products):
    for p in outer_products:
        outer = [operand[p](lambda e: block(2 * (e // 2) + a, 2 * (e % 2) + b)) for a in range(2) for b in range(2)]
        for q in range(7):
            yield 7 * p + q, operand[q](lambda e: outer[e])


def _transform_tables():
    theta = 2.0 * np.pi * np.arange(L)[:, None] * (np.arange(L)[None, :] + 1.0 / 3.0) / L
    forward = np.concatenate([np.cos(theta - np.pi / 6), np.sin(theta)], axis=1)
    inverse = np.concatenate([np.cos(theta + np.pi / 6).T, np.sin(theta).T], axis=1)
    return np.concatenate([forward, inverse * (2.0 / np.sqrt(3.0)) ** 3 / L], axis=0).astype(BF16)


def _dot(a, b):
    return jnp.dot(a, b, preferred_element_type=F32)


def _pack_rows(rows):
    return pltpu.bitcast(jnp.concatenate([rows[:8], rows[8:]], axis=1).astype(BF16).reshape(16, L), U32)


def _unpack_rows(x):
    u = pltpu.bitcast(x, U32)
    return jnp.concatenate([pltpu.bitcast(u << 16, F32), pltpu.bitcast(u & np.uint32(0xFFFF0000), F32)], axis=0)


def _geglu(a, b):
    ab = a * b
    return ab + ab * jnp.tanh(a * (GELU_LIN + a * a))


def _causal(k, u, init=None):
    acc = [t * u[0] for t in k]
    if init is not None:
        acc = [i + t for i, t in zip(init, acc)]
    for b in range(1, len(k)):
        for a in range(b, len(k)):
            acc[a] = acc[a] + k[a - b] * u[b]
    return acc


def _causal_halves(k, u):
    n = len(k) // 2
    upper = [k[n + a] * u[0] for a in range(n)]
    for b in range(1, n):
        upper = [upper[a] + k[n + a - b] * u[b] for a in range(n)]
    return _causal(k[:n], u[:n]) + _causal(k[:n], u[n:], upper)


def _block_product(w1, w2, u1, u2):
    t1 = _causal_halves([w1[0]] + [w1[b] + w2[b - 1] for b in range(1, NB)], u1)
    w3 = [a - b for a, b in zip(w1, w2)]
    t2 = _causal_halves([w2[0]] + [w2[b] - w3[b - 1] for b in range(1, NB)], u2)
    y1 = [a - b for a, b in zip(t1, t2)]
    t3 = _causal_halves([w3[0]] + [w3[b] + w1[b - 1] for b in range(1, NB)], [a - b for a, b in zip(u1, u2)])
    return y1, [a - b for a, b in zip(t1, t3)]


def _moments(total, squares):
    mean = jnp.sum(total, axis=0, keepdims=True) * (1.0 / D)
    var = jnp.maximum(jnp.sum(squares, axis=0, keepdims=True) * (1.0 / D) - mean * mean, 0.0)
    return mean, jax.lax.rsqrt(var + EPS)


def _interleave(first, first_count, second, second_count):
    streams = [[first, first_count, 0], [second, second_count, 0]]
    while streams:
        stream = min(streams, key=lambda s: (s[2] + 0.5) / s[1])
        stream[2] += 1
        if next(stream[0], _interleave) is _interleave:
            streams.remove(stream)


def _kernel(q_hbm, k_hbm, v_hbm, shift_hbm, filt_hbm, skip_hbm, wg_hbm, wu_hbm, wd_hbm, tab_hbm, out_hbm,
            xs, kb, vb, filt, shift, skip, wg, wu, wd, tab, par, ys, xm, wa, xb, hb, wc, sem):
    n_chunks = len(CONV_CHUNKS) - 1

    def copies(s, *pairs):
        return [pltpu.make_async_copy(src, dst, sem.at[s]) for src, dst in pairs]

    def conv_copies(c):
        rows = pl.ds(CONV_CHUNKS[c], CONV_CHUNKS[c + 1] - CONV_CHUNKS[c])
        pairs = [(src.at[rows], dst.at[rows]) for src, dst in ((filt_hbm, filt), (k_hbm, kb), (v_hbm, vb))]
        return copies(3 + c, *pairs, *([] if c else [(tab_hbm, tab)]))

    def out_copy(g, tile, count):
        cols = pl.ds(pl.multiple_of(g * G + tile * L, L), count * L)
        return pltpu.make_async_copy(xs.at[g, :, pl.ds(tile * L, count * L)], out_hbm.at[:, cols], sem.at[0])

    small_copies = copies(0, (shift_hbm, shift), (skip_hbm, skip))
    weight_copies = copies(1, (wg_hbm, wg), (wu_hbm, wu), (wd_hbm, wd))
    q_copies = copies(2, *[(q_hbm.at[:, pl.ds(g * G, G)], xs.at[g]) for g in range(NG)])
    for cp in small_copies + [cp for c in range(n_chunks) for cp in conv_copies(c)] + weight_copies + q_copies:
        cp.start()

    for i in range(49):
        xb[i, KQ // 2:, :] = jnp.zeros((L // 2 - KQ // 2, L), U32)
    for cp in small_copies:
        cp.wait()
    par[...] = jnp.concatenate([shift[...].astype(F32), skip[...].astype(F32).reshape(1, D),
                                jnp.zeros((3, D), F32)], axis=0).T

    def gated_signal(rows):
        lane = jax.lax.broadcasted_iota(jnp.int32, (SUB // 2, L), 1)
        coeffs = par[rows, :]
        taps = [jnp.broadcast_to(coeffs[:, j:j + 1], (SUB, L)) for j in range(4)]
        carry = [jnp.zeros((SUB // 2, L), U32)] * 4
        out = []
        for b in range(NB):
            if b % 2 == 0:
                v = vb[rows, b * L:(b + 2) * L].astype(F32)
            words = [pltpu.bitcast(kb[rows, b * L:(b + 1) * L], U32)]
            for j in range(1, 4):
                rolled = pltpu.roll(words[0], j, 1)
                words.append(jnp.where(lane < j, carry[j], rolled))
                carry[j] = rolled
            k = [pltpu.bitcast(t, BF16).astype(F32) for t in words]
            acc = taps[0] * k[0] + taps[1] * k[1] + taps[2] * k[2] + taps[3] * k[3]
            out.append(acc * v[:, (b % 2) * L:(b % 2 + 1) * L])
        return out

    spectra, results = [], []
    for s in range(D // SUB + 1):
        r0 = s * SUB
        if r0 < D:
            if r0 in CONV_CHUNKS:
                for cp in conv_copies(CONV_CHUNKS.index(r0)):
                    cp.wait()
            slabs = [pl.ds(r0 + e, 8) for e in range(0, SUB, 8)]
            wf = _dot(jnp.concatenate([filt[sl, b * L:(b + 1) * L] for sl in slabs for b in range(NB)], axis=0),
                      tab[:L, :])
            signal = gated_signal(pl.ds(r0, SUB))
            uf = _dot(jnp.concatenate([t[e:e + 8] for e in range(0, SUB, 8) for t in signal], axis=0).astype(BF16),
                      tab[:L, :])
            y1, y2 = [], []
            for e, sl in enumerate(slabs):
                coords = [[m[(e * NB + b) * 8:(e * NB + b + 1) * 8, h * L:(h + 1) * L] for b in range(NB)]
                          for m in (wf, uf) for h in range(2)]
                coords[0][0] = coords[0][0] + jnp.broadcast_to(par[sl, 4:5], (8, L)) * float(np.cos(np.pi / 6))
                a, b = _block_product(*coords)
                y1 += a
                y2 += b
            spectra.append((slabs, jnp.concatenate([jnp.concatenate(y1, axis=0), jnp.concatenate(y2, axis=0)],
                                                   axis=1).astype(BF16)))
        if s:
            slabs, spectrum = spectra.pop(0)
            results.append((slabs, _dot(spectrum, jnp.concatenate([tab[L:, :L], tab[L:, L:]], axis=0))))
        while len(results) > (1 if r0 < D else 0):
            slabs, y = results.pop(0)
            for t, (sl, b) in enumerate(itertools.product(slabs, range(NB))):
                ys[b // 4, sl, (b % 4) * L:(b % 4 + 1) * L] = y[8 * t:8 * t + 8]

    for cp in weight_copies:
        cp.wait()
    for c in range(FH // L):
        cols = [pl.ds(half * FH + c * L, L) for half in range(2)]
        for r in range(0, H, 16):
            quad = [wd[i * H + r:i * H + r + 16, cols[j]] for i in range(2) for j in range(2)]
            rows = [_unpack_rows(t) for t in quad]
            for i in range(7):
                wc[i, r // 2:r // 2 + 8, c * L:(c + 1) * L] = (
                    pltpu.bitcast(quad[3 * (i - 2)], U32) if i in (2, 3) else _pack_rows(_LEFT[i](lambda e: rows[e])))
        blocks = [[jnp.concatenate([ref[kq * KQ:(kq + 1) * KQ, col], jnp.zeros((L - KQ, L), BF16)], axis=0).T
                   for kq in range(4)] for ref in (wg, wu) for col in cols]
        for r in range(0, L, 16):
            rows = [[_unpack_rows(t[r:r + 16]) for t in row] for row in blocks]
            for i, value in _two_level(_LEFT, lambda a, b: rows[a][b], range(7)):
                if i // 7 in (2, 3) and i % 7 in (2, 3):
                    a = 2 * (i // 7 - 2) + i % 7 - 2
                    words = pltpu.bitcast(blocks[a][a][r:r + 16], U32)
                else:
                    words = _pack_rows(value)
                wa[i, (c * L + r) // 2:(c * L + r) // 2 + 8, :] = words

    def input_moments(g, stats):
        total = squares = None
        for r in range(0, D, 8):
            x = xs[g, r:r + 8, :].astype(F32)
            total, squares = (x, x * x) if r == 0 else (total + x, squares + x * x)
            if (r + 8) % RB == 0:
                yield
        stats.extend(_moments(total, squares))

    def apply_gate(g, g_read, stats):
        total = squares = None
        for r in range(0, D, 8):
            x = xs[g_read, r:r + 8, :].astype(F32)
            x = x + ((x - stats[0]) * stats[1]) * ys[g, r:r + 8, :]
            for j in range(4):
                xm[g, j, r:r + 8, :] = x[:, j * L:(j + 1) * L]
            total, squares = (x, x * x) if r == 0 else (total + x, squares + x * x)
            if (r + 8) % RB == 0:
                yield
        stats.extend(_moments(total, squares))

    def right_operands(g_read, stats, on_rows_done):
        scale = stats[3] * GELU_IN
        for r in range(0, KQ, 16):
            @functools.cache
            def z(kq, j):
                x = jnp.concatenate([xm[g_read, j, pl.ds(kq * KQ + r + e, 8, stride=2), :] for e in range(2)], axis=0)
                return (x - stats[2][:, j * L:(j + 1) * L]) * scale[:, j * L:(j + 1) * L]

            for t, (i, value) in enumerate(_two_level(_RIGHT, z, (1, 0, 4, 2, 5, 3, 6))):
                xb[i, r // 2:r // 2 + 8, :] = _pack_rows(value)
                if t == 48:
                    on_rows_done(r)
                if t % 7 == 6:
                    yield

    def gate_up():
        for r in range(0, FH, RC):
            m = [None] * 49
            for i in [7 * p + q for p in _ORDER for q in _ORDER]:
                m[i] = _dot(pltpu.bitcast(wa[i, r // 2:(r + RC) // 2, :], BF16), pltpu.bitcast(xb[i], BF16))
            inner = [_result_blocks(m[7 * p:7 * p + 7]) for p in range(7)]
            for t in range(0, RC, 16):
                h = {}
                for e in range(4):
                    c = _result_blocks([inner[p][e][t:t + 16] for p in range(7)])
                    h[e // 2, e % 2], h[e // 2, 2 + e % 2] = _geglu(c[0], c[2]), _geglu(c[1], c[3])
                blocks = [jnp.concatenate([h[a, 2 * j], h[a, 2 * j + 1]], axis=1) for a in range(2) for j in range(2)]
                for i in range(7):
                    hb[i, r + t:r + t + 16, :] = _RIGHT[i](lambda e: blocks[e]).astype(BF16)

    def down(g, on_progress, on_half_done):
        for n in range(2):
            def emit(i, j, value):
                rows, tile = slice(i * H, (i + 1) * H), 2 * j + n
                xs[g, rows, tile * L:(tile + 1) * L] = (xm[g, tile, rows, :] + GELU_OUT * value).astype(BF16)

            m = {}
            for i in _ORDER:
                for k0, k1 in ((0, 4 * L), (4 * L, FH)):
                    part = _dot(pltpu.bitcast(wc[i, :, k0:k1], BF16), hb[i, k0:k1, n * L:(n + 1) * L])
                    m[i] = m[i] + part if k0 else part
                    for r in range(0, H, H // 4):
                        on_progress(part[r:r + 8])
                        yield
                if i == (1 if n else 0):
                    emit(1, 0, m[1] + m[3])
                if i == (4 if n else 0):
                    emit(0, 1, m[2] + m[4])
                if i == 6:
                    emit(0, 0, m[3] - m[4] + m[0] + m[6])
                if i == 5:
                    emit(1, 1, m[2] - m[1] + m[0] + m[5])
            on_half_done(n)

    for cp in q_copies:
        cp.wait()
    first = []
    for _ in itertools.chain(input_moments(0, first), apply_gate(0, 0, first),
                             right_operands(0, first, lambda r: None)):
        pass

    def ffn_step(step, carry):
        g, nxt = step & (NG - 1), (step + 1) & (NG - 1)
        zero = [step >> 10, step >> 11]
        stats, deadlines, clock = [], [], [0]

        def on_progress(value):
            if len(stats) < 4:
                xs[zero[0] + NG, :8, :L] = value.astype(BF16)
            else:
                xm[zero[0] + NG, 0, :8, :] = value
            clock[0] += 1
            while deadlines and deadlines[0][0] <= clock[0]:
                hb[zero[0] + 7, :8, :L] = pltpu.bitcast(deadlines.pop(0)[1], F32).astype(BF16)

        def on_rows_done(r):
            deadlines.append((clock[0] + 12, xb[zero[0] + 42, r // 2:r // 2 + 8, :]))

        def on_half_done(n):
            @pl.when(step >= NG)
            def _():
                out_copy(g, n, 1).start()
                out_copy(g, 2 + n, 1).start()

        gate_up()
        products = down(g, on_progress, on_half_done)
        _interleave(itertools.islice(products, 12), 12, input_moments(nxt, stats), D // RB)
        _interleave(itertools.islice(products, 24), 24, apply_gate(nxt, nxt + zero[0], stats), D // RB)
        _interleave(products, 76, right_operands(nxt + zero[1], stats, on_rows_done), 49 * 1.4)
        return carry

    jax.lax.fori_loop(0, 2 * NG, ffn_step, 0)
    for g in range(NG):
        out_copy(g, 0, 4).wait()


@jax.jit
def pallas_interleave_layers__ssm_conv_h3__geglu_ffn__prompt_kernel(
    A_q: jax.Array,
    A_k: jax.Array,
    A_v: jax.Array,
    A_shift_k: jax.Array,
    A_ssm_k: jax.Array,
    A_ssm_D: jax.Array,
    B_x: jax.Array,
    B_w_gate: jax.Array,
    B_w_up: jax.Array,
    B_w_down: jax.Array,
):
    del B_x
    hbm = pl.BlockSpec(memory_space=pltpu.MemorySpace.HBM)
    out = pl.pallas_call(
        _kernel,
        out_shape=jax.ShapeDtypeStruct((D, S), BF16),
        in_specs=[hbm] * 10,
        out_specs=hbm,
        scratch_shapes=[
            pltpu.VMEM((NG + 1, D, G), BF16),
            pltpu.VMEM((D, S), BF16),
            pltpu.VMEM((D, S), BF16),
            pltpu.VMEM((D, S), BF16),
            pltpu.VMEM((4, D), BF16),
            pltpu.VMEM((D,), BF16),
            pltpu.VMEM((D, F), BF16),
            pltpu.VMEM((D, F), BF16),
            pltpu.VMEM((D, F), BF16),
            pltpu.VMEM((2 * L, 2 * L), BF16),
            pltpu.VMEM((D, 8), F32),
            pltpu.VMEM((NG, D, G), F32),
            pltpu.VMEM((NG + 1, 4, D + 8, L), F32),
            pltpu.VMEM((49, FH // 2, L), U32),
            pltpu.VMEM((49, L // 2, L), U32),
            pltpu.VMEM((8, FH, 2 * L), BF16),
            pltpu.VMEM((7, H // 2, FH), U32),
            pltpu.SemaphoreType.DMA((2 + len(CONV_CHUNKS),)),
        ],
        compiler_params=pltpu.CompilerParams(vmem_limit_bytes=100 * 2**20),
    )(A_q.reshape(S, D).T, A_k.reshape(S, D).T, A_v.reshape(S, D).T, A_shift_k.T, A_ssm_k, A_ssm_D,
      B_w_gate, B_w_up, B_w_down.T, _transform_tables())
    return out.T.reshape(1, S, D)
```

```python
import functools
import itertools

import numpy as np
import jax
import jax.numpy as jnp
import jax.experimental.pallas as pl
import jax.experimental.pallas.tpu as pltpu

BF16, F32, U32 = jnp.bfloat16, jnp.float32, jnp.uint32
S, D, F = 2048, 448, 1792
L = 128
NB = S // L
G = 4 * L
NG = S // G
KQ = D // 4
H, FH = D // 2, F // 2
SUB = 16
RC = 64
RB = 32
CONV_CHUNKS = (0, 16, 48, 112, 240, 448)
SHARED = 24
EPS = 1e-5

GELU_IN = float((np.sqrt(2.0 / np.pi) * 0.044715) ** (1.0 / 3.0))
GELU_LIN = float(np.sqrt(2.0 / np.pi) / GELU_IN)
GELU_OUT = 0.5 / GELU_IN ** 2

_LEFT = (lambda x: x(0) + x(3), lambda x: x(2) + x(3), lambda x: x(0), lambda x: x(3),
         lambda x: x(0) + x(1), lambda x: x(2) - x(0), lambda x: x(1) - x(3))
_RIGHT = (lambda x: x(0) + x(3), lambda x: x(0), lambda x: x(1) - x(3), lambda x: x(2) - x(0),
          lambda x: x(3), lambda x: x(0) + x(1), lambda x: x(2) + x(3))
_ORDER = (3, 1, 2, 4, 0, 6, 5)


def _result_blocks(m):
    return (m[3] - m[4] + m[0] + m[6], m[2] + m[4], m[3] + m[1], m[2] - m[1] + m[0] + m[5])


def _two_level(operand, block, outer_products):
    for p in outer_products:
        outer = [operand[p](lambda e: block(2 * (e // 2) + a, 2 * (e % 2) + b)) for a in range(2) for b in range(2)]
        for q in range(7):
            yield 7 * p + q, operand[q](lambda e: outer[e])


def _transform_tables():
    theta = 2.0 * np.pi * np.arange(L)[:, None] * (np.arange(L)[None, :] + 1.0 / 3.0) / L
    forward = np.concatenate([np.cos(theta - np.pi / 6), np.sin(theta)], axis=1)
    inverse = np.concatenate([np.cos(theta + np.pi / 6).T, np.sin(theta).T], axis=1)
    return np.concatenate([forward, inverse * (2.0 / np.sqrt(3.0)) ** 3 / L], axis=0).astype(BF16)


def _dot(a, b):
    return jnp.dot(a, b, preferred_element_type=F32)


def _pack_rows(rows):
    return pltpu.bitcast(jnp.concatenate([rows[:8], rows[8:]], axis=1).astype(BF16).reshape(16, L), U32)


def _unpack_rows(x):
    u = pltpu.bitcast(x, U32)
    return jnp.concatenate([pltpu.bitcast(u << 16, F32), pltpu.bitcast(u & np.uint32(0xFFFF0000), F32)], axis=0)


def _geglu(a, b):
    ab = a * b
    return ab + ab * jnp.tanh(a * (GELU_LIN + a * a))


def _causal(k, u):
    acc = [t * u[0] for t in k]
    for b in range(1, len(k)):
        for a in range(b, len(k)):
            acc[a] = acc[a] + k[a - b] * u[b]
    return acc


def _block_product(f1, f2, u1, u2):
    f3 = [a - b for a, b in zip(f1, f2)]
    k = ([f1[0]] + [f1[b] + f2[b - 1] for b in range(1, NB)],
         [f2[0]] + [f2[b] - f3[b - 1] for b in range(1, NB)],
         [f3[0]] + [f3[b] + f1[b - 1] for b in range(1, NB)])
    t1, t2, t3 = [_causal(a, b) for a, b in zip(k, (u1, u2, [a - b for a, b in zip(u1, u2)]))]
    return [a - b for a, b in zip(t1, t2)], [a - b for a, b in zip(t1, t3)]


def _moments(pivot, total, squares):
    offset = jnp.sum(total, axis=0, keepdims=True) * (1.0 / D)
    var = jnp.maximum(jnp.sum(squares, axis=0, keepdims=True) * (1.0 / D) - offset * offset, 0.0)
    return pivot + offset, jax.lax.rsqrt(var + EPS)


def _balance(wg, wu):
    norm_g, norm_u = [jnp.sum(jnp.sum(jnp.square(w.astype(F32)), axis=0, keepdims=True), axis=1, keepdims=True)
                      for w in (wg, wu)]
    ratio = jnp.sqrt(2.0 * norm_g / norm_u)
    ratio = jnp.where((ratio > 2.0 ** -30) & (ratio < 2.0 ** 30), ratio, 1.0)
    bits = pltpu.bitcast(jnp.broadcast_to(ratio, (8, L)), U32) & np.uint32(0x7F800000)
    return pltpu.bitcast(bits, F32)[:1], pltpu.bitcast(np.uint32(0x7F000000) - bits, F32)[:1]


def _interleave(first, first_count, second, second_count):
    streams = [[first, first_count, 0], [second, second_count, 0]]
    while streams:
        stream = min(streams, key=lambda s: (s[2] + 0.5) / s[1])
        stream[2] += 1
        if next(stream[0], _interleave) is _interleave:
            streams.remove(stream)


def _kernel(q_hbm, k_hbm, v_hbm, shift_hbm, filt_hbm, skip_hbm, wg_hbm, wu_hbm, wd_hbm, tab_hbm, out_hbm,
            xs, kb, vb, filt, shift, skip, wg, wu, wd, tab, par, out_scale, ys, xm, wa, xb, hb, wc, sem):
    n_chunks = len(CONV_CHUNKS) - 1

    def copies(s, *pairs):
        return [pltpu.make_async_copy(src, dst, sem.at[s]) for src, dst in pairs]

    def conv_copies(c):
        rows = pl.ds(CONV_CHUNKS[c], CONV_CHUNKS[c + 1] - CONV_CHUNKS[c])
        pairs = [(src.at[rows], dst.at[rows]) for src, dst in ((filt_hbm, filt), (k_hbm, kb), (v_hbm, vb))]
        return copies(3 + c, *pairs, *([] if c else [(tab_hbm, tab)]))

    def out_copy(g, tile):
        cols = pl.ds(pl.multiple_of(g * G + tile * L, L), L)
        return pltpu.make_async_copy(xs.at[g, :, pl.ds(tile * L, L)], out_hbm.at[:, cols], sem.at[0])

    small_copies = copies(3 + n_chunks, (shift_hbm, shift), (skip_hbm, skip))
    weight_copies = copies(1, (wg_hbm, wg), (wu_hbm, wu)) + copies(2, (wd_hbm, wd))
    q_copies = [copies(0 if g else 2, (q_hbm.at[:, pl.ds(g * G, G)], xs.at[g]))[0] for g in range(NG)]
    for cp in small_copies + [cp for c in range(n_chunks) for cp in conv_copies(c)] + weight_copies + q_copies:
        cp.start()

    for i in range(49):
        xb[i, KQ // 2:, :] = jnp.zeros((L // 2 - KQ // 2, L), U32)
    for cp in small_copies:
        cp.wait()
    par[...] = jnp.concatenate([shift[...].astype(F32), skip[...].astype(F32).reshape(1, D),
                                jnp.zeros((3, D), F32)], axis=0).T

    def gated_signal(rows):
        lane = jax.lax.broadcasted_iota(jnp.int32, (SUB // 2, L), 1)
        coeffs = par[rows, :]
        taps = [jnp.broadcast_to(coeffs[:, j:j + 1], (SUB, L)) for j in range(4)]
        carry = [jnp.zeros((SUB // 2, L), U32)] * 4
        out = []
        for b in range(NB):
            if b % 2 == 0:
                v = vb[rows, b * L:(b + 2) * L].astype(F32)
            words = [pltpu.bitcast(kb[rows, b * L:(b + 1) * L], U32)]
            for j in range(1, 4):
                rolled = pltpu.roll(words[0], j, 1)
                words.append(jnp.where(lane < j, carry[j], rolled))
                carry[j] = rolled
            k = [pltpu.bitcast(t, BF16).astype(F32) for t in words]
            acc = (taps[0] * k[0] + taps[1] * k[1]) + (taps[2] * k[2] + taps[3] * k[3])
            out.append(acc * v[:, (b % 2) * L:(b % 2 + 1) * L])
        return out

    def spectrum(s):
        slabs = [pl.ds(s * SUB + e, 8) for e in range(0, SUB, 8)]
        wf = _dot(jnp.concatenate([filt[sl, b * L:(b + 1) * L] for sl in slabs for b in range(NB)], axis=0),
                  tab[:L, :])
        signal = gated_signal(pl.ds(s * SUB, SUB))
        uf = _dot(jnp.concatenate([t[e:e + 8] for e in range(0, SUB, 8) for t in signal], axis=0).astype(BF16),
                  tab[:L, :])
        y1, y2 = [], []
        for e, sl in enumerate(slabs):
            coords = [[m[(e * NB + b) * 8:(e * NB + b + 1) * 8, h * L:(h + 1) * L] for b in range(NB)]
                      for m in (wf, uf) for h in range(2)]
            coords[0][0] = coords[0][0] + jnp.broadcast_to(par[sl, 4:5], (8, L)) * float(np.cos(np.pi / 6))
            a, b = _block_product(*coords)
            y1 += a
            y2 += b
        return jnp.concatenate([jnp.concatenate(y1, axis=0), jnp.concatenate(y2, axis=0)], axis=1).astype(BF16)

    def interpolate(s, values):
        y = _dot(values, jnp.concatenate([tab[L:, :L], tab[L:, L:]], axis=0))
        for t, (e, b) in enumerate(itertools.product(range(0, SUB, 8), range(NB))):
            ys[b // 4, pl.ds(s * SUB + e, 8), (b % 4) * L:(b % 4 + 1) * L] = y[8 * t:8 * t + 8]

    def conv_pass(s, previous):
        current = spectrum(s)
        interpolate(s - 1, previous)
        return current

    def gate_up_weights(c, up_scale):
        cols = [pl.ds(half * FH + c * L, L) for half in range(2)]
        blocks = [[jnp.concatenate([ref[kq * KQ:(kq + 1) * KQ, col], jnp.zeros((L - KQ, L), BF16)], axis=0).T
                   for kq in range(4)] for ref in (wg, wu) for col in cols]
        for r in range(0, L, 16):
            rows = [[_unpack_rows(t[r:r + 16]) for t in row] for row in blocks]
            rows[2:] = [[t * up_scale for t in row] for row in rows[2:]]
            for i, value in _two_level(_LEFT, lambda a, b: rows[a][b], (2, 5, 4, 0, 3, 1, 6)):
                if i in (16, 17):
                    words = pltpu.bitcast(blocks[i - 16][i - 16][r:r + 16], U32)
                else:
                    words = _pack_rows(value)
                wa[i, pl.ds(c * (L // 2) + r // 2, 8), :] = words

    for c in range(n_chunks):
        for cp in conv_copies(c):
            cp.wait()
        lo, hi = CONV_CHUNKS[c] // SUB, min(CONV_CHUNKS[c + 1] // SUB, SHARED)
        pending = jax.lax.fori_loop(lo, hi, conv_pass, pending, unroll=True) if c else spectrum(0)

    for cp in weight_copies[:2]:
        cp.wait()
    up_scale, up_unscale = _balance(wg[:, :L], wu[:, :L])
    out_scale[...] = jnp.broadcast_to(GELU_OUT * up_unscale, (8, L))

    def shared_pass(s, previous):
        current = conv_pass(s, previous)
        gate_up_weights(s - SHARED, up_scale)
        return current

    interpolate(D // SUB - 1, jax.lax.fori_loop(SHARED, D // SUB, shared_pass, pending, unroll=True))
    pl.loop(D // SUB - SHARED, FH // L, unroll=True)(lambda c: gate_up_weights(c, up_scale))

    for cp in weight_copies[2:] + q_copies[:1]:
        cp.wait()

    @pl.loop(0, H // 16, unroll=True)
    def _(r):
        for c in range(0, FH, L):
            quad = [wd[pl.ds(i * H + r * 16, 16), j * FH + c:j * FH + c + L] for i in range(2) for j in range(2)]
            rows = [_unpack_rows(t) for t in quad]
            for i in range(7):
                wc[i, pl.ds(r * 8, 8), c:c + L] = (
                    pltpu.bitcast(quad[3 * (i - 2)], U32) if i in (2, 3) else _pack_rows(_LEFT[i](lambda e: rows[e])))

    def input_moments(g, stats):
        total = squares = None
        for r in range(0, D, 8):
            x = xs[g, r:r + 8, :].astype(F32)
            if r == 0:
                pivot = x[:1]
            d = x - pivot
            total, squares = (d, d * d) if r == 0 else (total + d, squares + d * d)
            if (r + 8) % RB == 0:
                yield
        stats.extend(_moments(pivot, total, squares))

    def apply_gate(g, g_read, stats):
        total = squares = None
        for r in range(0, D, 8):
            x = xs[g_read, r:r + 8, :].astype(F32)
            x = x + ((x - stats[0]) * stats[1]) * ys[g, r:r + 8, :]
            for j in range(4):
                xm[g, j, r:r + 8, :] = x[:, j * L:(j + 1) * L]
            if r == 0:
                pivot = x[:1]
            d = x - pivot
            total, squares = (d, d * d) if r == 0 else (total + d, squares + d * d)
            if (r + 8) % RB == 0:
                yield
        stats.extend(_moments(pivot, total, squares))

    def right_operands(g_read, stats, on_rows_done):
        scale = stats[3] * GELU_IN
        for r in range(0, KQ, 16):
            @functools.cache
            def z(kq, j):
                x = jnp.concatenate([xm[g_read, j, pl.ds(kq * KQ + r + e, 8, stride=2), :] for e in range(2)], axis=0)
                return (x - stats[2][:, j * L:(j + 1) * L]) * scale[:, j * L:(j + 1) * L]

            for t, (i, value) in enumerate(_two_level(_RIGHT, z, (1, 0, 4, 2, 5, 3, 6))):
                xb[i, r // 2:r // 2 + 8, :] = _pack_rows(value)
                if t == 48:
                    on_rows_done(r)
                if t % 7 == 6:
                    yield

    def gate_up():
        @pl.loop(0, FH // RC, unroll=True)
        def _(chunk):
            m = [None] * 49
            for i in [7 * p + q for p in _ORDER for q in _ORDER]:
                m[i] = _dot(pltpu.bitcast(wa[i, pl.ds(chunk * (RC // 2), RC // 2), :], BF16),
                            pltpu.bitcast(xb[i], BF16))
            inner = [_result_blocks(m[7 * p:7 * p + 7]) for p in range(7)]
            for t in range(0, RC, 16):
                h = {}
                for e in range(4):
                    c = _result_blocks([inner[p][e][t:t + 16] for p in range(7)])
                    h[e // 2, e % 2], h[e // 2, 2 + e % 2] = _geglu(c[0], c[2]), _geglu(c[1], c[3])
                blocks = [jnp.concatenate([h[a, 2 * j], h[a, 2 * j + 1]], axis=1) for a in range(2) for j in range(2)]
                for i in range(7):
                    hb[i, pl.ds(chunk * RC + t, 16), :] = _RIGHT[i](lambda e: blocks[e]).astype(BF16)

    def down(g, on_progress, on_tiles_done):
        for n in range(2):
            def emit(i, j, value):
                rows, tile = slice(i * H, (i + 1) * H), 2 * j + n
                xs[g, rows, tile * L:(tile + 1) * L] = (xm[g, tile, rows, :] + out_scale[:1] * value).astype(BF16)

            m = {}
            for i in _ORDER:
                for k0, k1 in ((0, 4 * L), (4 * L, FH)):
                    part = _dot(pltpu.bitcast(wc[i, :, k0:k1], BF16), hb[i, k0:k1, n * L:(n + 1) * L])
                    m[i] = m[i] + part if k0 else part
                    for r in range(0, H, H // 4):
                        on_progress(part[r:r + 8])
                        yield
                if i == (1 if n else 0):
                    emit(1, 0, m[1] + m[3])
                if i == (4 if n else 0):
                    emit(0, 1, m[2] + m[4])
                if i == 6:
                    emit(0, 0, m[3] - m[4] + m[0] + m[6])
                    if n:
                        on_tiles_done(1)
                if i == 5:
                    emit(1, 1, m[2] - m[1] + m[0] + m[5])
            on_tiles_done(*((3,) if n else (0, 2)))

    first = []
    for _ in itertools.chain(input_moments(0, first), apply_gate(0, 0, first),
                             right_operands(0, first, lambda r: None)):
        pass
    for cp in q_copies[1:]:
        cp.wait()

    def ffn_step(step, carry):
        g, nxt = step & (NG - 1), (step + 1) & (NG - 1)
        zero = [step >> 10, step >> 11]
        stats, deadlines, clock = [], [], [0]

        def on_progress(value):
            if len(stats) < 4:
                xs[zero[0] + NG, :8, :L] = value.astype(BF16)
            else:
                xm[zero[0] + NG, 0, :8, :] = value
            clock[0] += 1
            while deadlines and deadlines[0][0] <= clock[0]:
                hb[zero[0] + 7, :8, :L] = pltpu.bitcast(deadlines.pop(0)[1], F32).astype(BF16)

        def on_rows_done(r):
            deadlines.append((clock[0] + 10, xb[zero[0] + 42, r // 2:r // 2 + 8, :]))

        def on_tiles_done(*tiles):
            @pl.when(step >= NG)
            def _():
                for tile in tiles:
                    out_copy(g, tile).start()

        gate_up()
        products = down(g, on_progress, on_tiles_done)
        _interleave(itertools.islice(products, 12), 12, input_moments(nxt, stats), D // RB)
        _interleave(itertools.islice(products, 24), 24, apply_gate(nxt, nxt + zero[0], stats), D // RB)
        _interleave(products, 76, right_operands(nxt + zero[1], stats, on_rows_done), 49 * 1.4)
        return carry

    jax.lax.fori_loop(0, 2 * NG, ffn_step, 0)
    for g, tile in itertools.product(range(NG), range(4)):
        out_copy(g, tile).wait()


@jax.jit
def pallas_interleave_layers__ssm_conv_h3__geglu_ffn__prompt_kernel(
    A_q: jax.Array,
    A_k: jax.Array,
    A_v: jax.Array,
    A_shift_k: jax.Array,
    A_ssm_k: jax.Array,
    A_ssm_D: jax.Array,
    B_x: jax.Array,
    B_w_gate: jax.Array,
    B_w_up: jax.Array,
    B_w_down: jax.Array,
):
    del B_x
    hbm = pl.BlockSpec(memory_space=pltpu.MemorySpace.HBM)
    out = pl.pallas_call(
        _kernel,
        out_shape=jax.ShapeDtypeStruct((D, S), BF16),
        in_specs=[hbm] * 10,
        out_specs=hbm,
        scratch_shapes=[
            pltpu.VMEM((NG + 1, D, G), BF16),
            pltpu.VMEM((D, S), BF16),
            pltpu.VMEM((D, S), BF16),
            pltpu.VMEM((D, S), BF16),
            pltpu.VMEM((4, D), BF16),
            pltpu.VMEM((D,), BF16),
            pltpu.VMEM((D, F), BF16),
            pltpu.VMEM((D, F), BF16),
            pltpu.VMEM((D, F), BF16),
            pltpu.VMEM((2 * L, 2 * L), BF16),
            pltpu.VMEM((D, 8), F32),
            pltpu.VMEM((8, L), F32),
            pltpu.VMEM((NG, D, G), F32),
            pltpu.VMEM((NG + 1, 4, D + 8, L), F32),
            pltpu.VMEM((49, FH // 2, L), U32),
            pltpu.VMEM((49, L // 2, L), U32),
            pltpu.VMEM((8, FH, 2 * L), BF16),
            pltpu.VMEM((7, H // 2, FH), U32),
            pltpu.SemaphoreType.DMA((3 + len(CONV_CHUNKS),)),
        ],
        compiler_params=pltpu.CompilerParams(vmem_limit_bytes=100 * 2**20),
    )(A_q.reshape(S, D).T, A_k.reshape(S, D).T, A_v.reshape(S, D).T, A_shift_k.T, A_ssm_k, A_ssm_D,
      B_w_gate, B_w_up, B_w_down.T, _transform_tables())
    return out.T.reshape(1, S, D)
```
